```python
import os as _os
_os.environ.setdefault("JAX_PLATFORMS", "cpu")
import jax
import jax.numpy as jnp

def _softmax(x, axis=-1):
    return jax.nn.softmax(x, axis=axis)
def _gelu(x):
    return jax.nn.gelu(x, approximate=True)
def _silu(x):
    return jax.nn.silu(x)
def _sigmoid(x):
    return jax.nn.sigmoid(x)
def _layernorm(x, axis=-1, eps=1e-5):
    m = jnp.mean(x, axis=axis, keepdims=True)
    v = jnp.var(x, axis=axis, keepdims=True)
    return (x - m) / jnp.sqrt(v + eps)
def _scatter_add(tgt, idx, src, axis=0):
    return tgt.at[idx].add(src)
def _segment_sum(src, seg, n):
    return jax.ops.segment_sum(src, seg, n)
class _Rng:
    def __init__(self, key):
        self._k = key
    def _next(self):
        self._k, sub = jax.random.split(self._k)
        return sub
    def normal(self, shape):
        return jax.random.normal(self._next(), shape, dtype=jnp.bfloat16)
    def randint(self, lo, hi, shape):
        return jax.random.randint(self._next(), shape, lo, hi, dtype=jnp.int32)
    def uniform(self, shape, lo=0.0, hi=1.0):
        return jax.random.uniform(self._next(), shape, jnp.bfloat16, lo, hi)
    def permutation(self, n):
        return jax.random.permutation(self._next(), n)


kernel_name = 'parallel_sum__sliding_local_dilated__dense_activation_mish__prompt'

def setup_inputs():
    _rng = _Rng(jax.random.key(int.from_bytes(__import__("os").urandom(4), "little")))
    _w = (lambda a: (lambda t: t.astype(jnp.bfloat16) if jnp.issubdtype(t.dtype, jnp.floating) else t)(jnp.asarray(a)))
    def _A_setup():
        B, S, D = 1, 2048, 576
        return {
            "x": _w((lambda *s: _rng.normal(s) * 0.05)(B, S, D)),
            "wqkv": _w((lambda *s: _rng.normal(s) * 0.05)(D, 3 * D)),
            "wo": _w((lambda *s: _rng.normal(s) * 0.05)(D, D)),
        }
    _A_in = _A_setup()

    def _B_setup():
        B, S, D, F = 1, 2048, 576, 4608
        return {
            "x": _w((lambda *s: _rng.normal(s) * 0.05)(B, S, D)),
            "w1": _w((lambda *s: _rng.normal(s) * 1.6)(D, F) * (D ** -0.5)),
            "b1": _w((lambda *s: _rng.normal(s) * 0.2)(F)),
            "w2": _w((lambda *s: _rng.normal(s) * 0.2)(F, D) * (F ** -0.5)),
        }
    _B_in = _B_setup()

    return {
        "A_x": _A_in["x"],
        "A_wqkv": _A_in["wqkv"],
        "A_wo": _A_in["wo"],
        "B_x": _B_in["x"],
        "B_w1": _B_in["w1"],
        "B_b1": _B_in["b1"],
        "B_w2": _B_in["w2"],
    }

def reference(A_x, A_wqkv, A_wo, B_x, B_w1, B_b1, B_w2):
    def _A_ref(x, wqkv, wo):
        B, S, D = x.shape
        H = 32; Dh = D // H
        W, dil = 8, 2
        qkv = (lambda x, *d: x.transpose(*d))((x @ wqkv).reshape(B, S, 3, H, Dh), 2, 0, 3, 1, 4)
        q, k, v = qkv[0], qkv[1], qkv[2]
        scale = Dh ** -0.5
        pos = jnp.arange(S)
        off = jnp.arange(W) * dil
        idx = pos[:, None] - off[None, :]
        mask = idx >= 0
        idx_c = jnp.where(mask, idx, 0).reshape(-1)
        kg = k[:, :, idx_c, :].reshape(B, H, S, W, Dh)
        vg = v[:, :, idx_c, :].reshape(B, H, S, W, Dh)
        logits = jnp.einsum("bhsd,bhswd->bhsw", q, kg) * scale
        logits = jnp.where(mask[None, None, :, :], logits, -1e9)
        attn = _softmax(logits, axis=-1)
        o = jnp.einsum("bhsw,bhswd->bhsd", attn, vg)
        return (lambda x, *d: x.transpose(*d))(o, 0, 2, 1, 3).reshape(B, S, D) @ wo

    def _B_ref(x, w1, b1, w2):
        h = jnp.einsum("bsd,df->bsf", x, w1) + b1
        sp = jnp.log1p(jnp.exp(-jnp.abs(h))) + jnp.where(h > 0, h, jnp.zeros_like(h))
        act = h * jnp.tanh(sp)
        return jnp.einsum("bsf,fd->bsd", act, w2)

    x = A_x
    xn = _layernorm(x, axis=-1)
    return x + _A_ref(xn, A_wqkv, A_wo) + _B_ref(xn, B_w1, B_b1, B_w2)
```

```python
import contextlib
import os
import jax
import jax.numpy as jnp
from jax import lax
import jax.experimental.pallas as pl
import jax.experimental.pallas.tpu as pltpu

S, D, F = 2048, 576, 4608
DP = 640
FC = 512
NC = F // FC
TT = 256
NTT = S // TT
H, DH, WIN, DIL = 32, 18, 8, 2
HALO = 16
NSLAB = 14
EPS = 1e-5
LOG2E = 1.4426950408889634
SCALE = DH ** -0.5
NT = (((1,), (1,)), ((), ()))
RC = int(os.environ.get("RC", "8"))
ATT_SPREAD = int(os.environ.get("ATT_SPREAD", "7"))
GATE = int(os.environ.get("GATE", "1"))
CHAIN = int(os.environ.get("CHAIN", "1"))
PREP_AT = int(os.environ.get("PREP_AT", "2"))
SCOPES = bool(int(os.environ.get("SCOPES", "0")))
F32 = jnp.float32
BF16 = jnp.bfloat16

NSEM = 6
SPLITW = int(os.environ.get('SPLITW', '1'))
XG = 2
NSPL = int(os.environ.get("NSPL", "4"))
GATE_U = int(os.environ.get("GATE_U", "3"))
OSPLIT = int(os.environ.get("OSPLIT", "4"))


def scope(name):
    return jax.named_scope(name) if SCOPES else contextlib.nullcontext()


def _mish(h):
    e = jnp.exp(jnp.minimum(h, 20.0))
    n = e * (e + 2.0)
    return (h * n) * pl.reciprocal(n + 2.0, approx=True)


def _never(v):
    return jnp.minimum(pltpu.bitcast(v, jnp.int32), 5) > 7


def _kernel(x_hbm, wqkv_hbm, wo_hbm, w1_hbm, b1_hbm, w2_hbm, out_hbm,
            x_s, xn_s, w1_s, w2_s, wqkv_s, wo_s, wt_s, wot_s, slab_s,
            act_s, acc_s, qkv_s, o_s, out_s, b1_s, stg_s, sems):

    def rows(j, n=TT):
        if isinstance(j, int):
            return pl.ds(j * n, n)
        return pl.ds(pl.multiple_of(j * n, n), n)

    def x_copy(j, sem):
        return pltpu.make_async_copy(x_hbm.at[:, rows(j)], x_s.at[j], sems.at[sem])

    def w1_copy(c, sem):
        return pltpu.make_async_copy(w1_hbm.at[:, rows(c, FC)],
                                     w1_s.at[c, pl.ds(0, D), :], sems.at[sem])

    def w2_copy(c, sem):
        return pltpu.make_async_copy(w2_hbm.at[:, rows(c, FC)], w2_s.at[c], sems.at[sem])

    def out_copy(j, r0, nr):
        return pltpu.make_async_copy(out_s.at[j, pl.ds(r0, nr), :],
                                     out_hbm.at[pl.ds(r0, nr), rows(j)], sems.at[0])

    wqkv_copy = pltpu.make_async_copy(wqkv_hbm, wqkv_s, sems.at[1])
    wo_copy = pltpu.make_async_copy(wo_hbm, wo_s, sems.at[1])
    b1_copy = pltpu.make_async_copy(b1_hbm, b1_s, sems.at[0])

    def w1_half(h, sem):
        hw = FC // 2
        return pltpu.make_async_copy(w1_hbm.at[:, pl.ds(h * hw, hw)],
                                     w1_s.at[0, pl.ds(0, D), pl.ds(h * hw, hw)], sems.at[sem])

    def ffn1(j, c, nsplit=1, src=None, gate=None, parts=None):
        nw = FC // nsplit
        for u in (range(nsplit) if parts is None else parts):
            lhs = xn_s[rows(j), :] if src is None else src[...]
            if gate is not None and u == GATE_U:
                head = pltpu.bitcast(lhs[0:16, 0:128], jnp.int32)
                head = pltpu.bitcast(jnp.where(gate, 0, head), BF16)
                top = jnp.concatenate([head, lhs[0:16, 128:]], axis=1)
                lhs = jnp.concatenate([top, lhs[16:, :]], axis=0)
            h = jnp.dot(lhs, w1_s[c, :, u * nw:(u + 1) * nw], preferred_element_type=F32)
            act_s[rows(j), u * nw:(u + 1) * nw] = _mish(h).astype(BF16)

    def ffn2(j, c):
        return lax.dot_general(w2_s[c], act_s[rows(j), :], NT, preferred_element_type=F32)

    def layernorm(j, stage=None):
        rowp = lax.broadcasted_iota(jnp.int32, (DP - D, TT), 0)
        ones_pad = jnp.where(rowp == 0, 1.0, 0.0).astype(F32)
        xt = x_s[j].astype(F32)
        m = jnp.sum(xt, axis=0, keepdims=True) * (1.0 / D)
        xc = xt - m
        v = jnp.sum(xc * xc, axis=0, keepdims=True) * (1.0 / D)
        xn = xc * lax.rsqrt(v + EPS)
        xn = jnp.concatenate([xn, ones_pad], axis=0)
        xnb = xn.T.astype(BF16)
        xn_s[rows(j), :] = xnb
        if stage is not None:
            stage[...] = xnb
        g = None
        for r0 in range(112, TT, 128):
            for c0 in range(0, DP, 128):
                blk = pltpu.bitcast(xnb[r0:r0 + 16, c0:c0 + 128], jnp.int32)
                g = blk if g is None else jnp.minimum(g, blk)
        return jnp.minimum(g, 5) > 7

    def bias_rows(c):
        b = b1_s[...].astype(F32)
        row16 = lax.broadcasted_iota(jnp.int32, (16, 128), 0)
        for u in range(FC // 128):
            r = c * (FC // 128) + u
            w1_s[c, D:D + 16, u * 128:(u + 1) * 128] = jnp.where(
                row16 == 0, jnp.broadcast_to(b[r:r + 1, :], (16, 128)), 0.0).astype(BF16)

    def prep_weights():
        for c in range(5):
            nr = 128 if c < 4 else 64
            blk = wqkv_s[c * 128:c * 128 + nr, :].astype(F32)
            if nr < 128:
                blk = jnp.concatenate([blk, jnp.zeros((128 - nr, 3 * D), F32)], axis=0)
            slab_s[c, 0:3 * D, :] = blk.T
        for t in range(3):
            for d in range(DH):
                if d < 16:
                    dst = t * 512 + d * H
                else:
                    dst = {0: 1536, 2: 1600, 1: 1664}[t] + (d - 16) * H
                wt_s[dst:dst + H, :] = jnp.concatenate(
                    [slab_s[c, pl.ds(t * D + d, H, stride=DH), :] for c in range(5)],
                    axis=1).astype(BF16)
        for c in range(5):
            cols = 128 if c < 4 else 64
            blk = wo_s[:, c * 128:c * 128 + cols].astype(F32)
            if cols < 128:
                blk = jnp.concatenate([blk, jnp.zeros((D, 128 - cols), F32)], axis=1)
            slab_s[c, 3 * D:4 * D, :] = blk
        for c in range(5):
            nr = 128 if c < 4 else 64
            parts = [slab_s[c, pl.ds(3 * D + d, H, stride=DH), :] for d in range(16)]
            parts.append(jnp.zeros((64, 128), F32))
            parts += [slab_s[c, pl.ds(3 * D + d, H, stride=DH), :] for d in (16, 17)]
            p = jnp.concatenate(parts, axis=0)
            pt = p.T[:nr, :]
            wot_s[c * 128:c * 128 + nr, :] = pt.astype(BF16)
            g = pltpu.bitcast(pt[nr - 8:nr, 0:128], jnp.int32)
            for bb in range(1, 5):
                g = jnp.minimum(g, pltpu.bitcast(pt[nr - 8:nr, bb * 128:(bb + 1) * 128], jnp.int32))
            z = jnp.where(jnp.minimum(g, 5) > 7, 1.0, 0.0)
            wt_s[3 * D:NSLAB * 128, c * 128:(c + 1) * 128] = jnp.concatenate(
                [z] * 8, axis=0).astype(BF16)

    q_sl = (0, 1, 2, 3, 12)
    k_sl = (4, 5, 6, 7, 13)
    v_sl = (8, 9, 10, 11, 12)

    def attention_rows(t, r, gate):
        q = [qkv_s[sl, HALO + r:HALO + r + RC, :] for sl in q_sl]
        if gate is not None:
            q = [jnp.where(gate, 0.0, qq) for qq in q]
        ls = []
        for w in range(WIN):
            o0 = HALO + r - DIL * w
            s = q[0] * qkv_s[k_sl[0], o0:o0 + RC, :]
            for jj in range(1, 5):
                s = s + q[jj] * qkv_s[k_sl[jj], o0:o0 + RC, :]
            s = s + pltpu.roll(s, 64, 1)
            s = s + pltpu.roll(s, 32, 1)
            if r < HALO and w > 0:
                pos = t * TT + r + lax.broadcasted_iota(jnp.int32, (RC, 128), 0)
                s = jnp.where(pos >= DIL * w, s, -1e9 / SCALE)
            ls.append(s)
        m = ls[0]
        for w in range(1, WIN):
            m = jnp.maximum(m, ls[w])
        ps = [jnp.exp2((l - m) * (SCALE * LOG2E)) for l in ls]
        den = ps[0]
        for w in range(1, WIN):
            den = den + ps[w]
        rinv = pl.reciprocal(den, approx=True)
        outs = []
        for jj in range(5):
            a = ps[0] * qkv_s[v_sl[jj], HALO + r:HALO + r + RC, :]
            for w in range(1, WIN):
                o0 = HALO + r - DIL * w
                a = a + ps[w] * qkv_s[v_sl[jj], o0:o0 + RC, :]
            outs.append(a * rinv)
        o_s[r:r + RC, :] = jnp.concatenate(outs, axis=1).astype(BF16)
        return den

    def attention_group(t, rs, src):
        gate = _never(src[0:RC, 0:128]) if GATE else None
        for r in rs:
            den = attention_rows(t, r, gate)
            if CHAIN:
                gate = _never(den)

    def qkv_proj(t):
        qkv_s[4:NSLAB, 0:HALO, :] = qkv_s[4:NSLAB, TT:TT + HALO, :]
        qkv = lax.dot_general(xn_s[rows(t), :], wt_s[...], NT, preferred_element_type=F32)
        for sl in range(NSLAB):
            qkv_s[sl, HALO:HALO + TT, :] = qkv[:, sl * 128:(sl + 1) * 128]

    def wo_proj():
        return lax.dot_general(wot_s[...], o_s[...], NT, preferred_element_type=F32)

    chunks = list(range(0, TT, RC))
    att_sched = [[] for _ in range(NTT)]
    for i, r in enumerate(chunks):
        att_sched[i * ATT_SPREAD // len(chunks)].append(r)

    with scope("step0a"):
        x_copy(0, 0).start()
        b1_copy.start()
        if SPLITW:
            w1_half(0, 5).start()
            x_copy(1, 1).start()
            w1_half(1, 1).start()
        else:
            w1_copy(0, 1).start()
            x_copy(1, 1).start()
        for j in range(2, NTT):
            x_copy(j, 2 + (j - 2) // XG).start()
        if not SPLITW:
            w1_copy(1, 5).start()
            w2_copy(0, 5).start()
        for c in range(NC):
            w1_s[c, D + 16:DP, :] = jnp.zeros((DP - D - 16, FC), BF16)
        qkv_s[:, TT:TT + HALO, :] = jnp.zeros((NSLAB, HALO, 128), F32)

        x_copy(0, 0).wait()
        b1_copy.wait()
        layernorm(0)
        for c in range(NC):
            bias_rows(c)
        if SPLITW:
            w1_half(0, 5).wait()
            w1_copy(1, 5).start()
            w2_copy(0, 5).start()
            ffn1(0, 0, nsplit=4, parts=(0, 1))
            x_copy(1, 1).wait()
            w1_half(1, 1).wait()
            wqkv_copy.start()
            wo_copy.start()
            g = layernorm(1, stg_s.at[XG - 1])
            ffn1(0, 0, nsplit=4, parts=(2, 3))
        else:
            w1_copy(0, 1).wait()
            x_copy(1, 1).wait()
            wqkv_copy.start()
            wo_copy.start()
            g = layernorm(1, stg_s.at[XG - 1])
            ffn1(0, 0, nsplit=NSPL, gate=g)

    def step0(i, carry):
        with scope("step0b"):
            for u in range(XG):
                x_copy(XG * i + 2 + u, 2 + i).wait()
            for u in range(XG):
                g = layernorm(XG * i + 2 + u, stg_s.at[u])
                ffn1(XG * i + 1 + u, 0, nsplit=NSPL, src=stg_s.at[(u - 1) % XG], gate=g)
        return carry

    lax.fori_loop(0, (NTT - 2) // XG, step0, 0)

    with scope("step1"):
        w1_copy(1, 5).wait()
        w2_copy(0, 5).wait()
        w1_copy(2, 2).start()
        w2_copy(1, 2).start()
        ffn1(NTT - 1, 0)
        for j in range(NTT):
            acc_s[j] = x_s[j].astype(F32) + ffn2(j, 0)
            if j == PREP_AT:
                wqkv_copy.wait()
                wo_copy.wait()
                prep_weights()
            ffn1(j, 1)
        qkv_proj(0)

    def step(s, carry):
        with scope("steady"):
            t = s - 2
            cur = 2 + lax.rem(s, 2)
            nxt = 5 - cur
            w1_copy(s, cur).wait()
            w2_copy(s - 1, cur).wait()
            w2_copy(s, nxt).start()

            @pl.when(s + 1 < NC)
            def _():
                w1_copy(s + 1, nxt).start()

            for j in range(NTT):
                y = ffn2(j, s - 1)
                acc_s[j] += y
                ffn1(j, s)
                if att_sched[j]:
                    attention_group(t, att_sched[j], y)
            acc_s[t] += wo_proj()
            qkv_proj(t + 1)
        return carry

    lax.fori_loop(2, NC, step, 0)

    with scope("last"):
        w2_copy(NC - 1, 2 + NC % 2).wait()
        t = NTT - 1
        outs = []
        for j in range(NTT):
            y = ffn2(j, NC - 1)
            res = acc_s[j] + y
            if j == t:
                res = res + wo_proj()
            nsp = OSPLIT if j == t else 1
            nr = D // nsp
            for u in range(nsp):
                out_s[j, u * nr:(u + 1) * nr, :] = res[u * nr:(u + 1) * nr, :].astype(BF16)
                cp = out_copy(j, u * nr, nr)
                cp.start()
                outs.append(cp)
            if att_sched[j]:
                attention_group(t, att_sched[j], y)
        for cp in outs:
            cp.wait()


@jax.jit
def pallas_parallel_sum__sliding_local_dilated__dense_activation_mish__prompt_kernel(
    A_x, A_wqkv, A_wo, B_x, B_w1, B_b1, B_w2):
    del B_x
    xT = jnp.transpose(A_x, (0, 2, 1)).reshape(D, S)
    any_spec = pl.BlockSpec(memory_space=pl.ANY)
    outT = pl.pallas_call(
        _kernel,
        out_shape=jax.ShapeDtypeStruct((D, S), BF16),
        in_specs=[any_spec] * 6,
        out_specs=any_spec,
        scratch_shapes=[
            pltpu.VMEM((NTT, D, TT), BF16),
            pltpu.VMEM((S, DP), BF16),
            pltpu.VMEM((NC, DP, FC), BF16),
            pltpu.VMEM((NC, D, FC), BF16),
            pltpu.VMEM((D, 3 * D), BF16),
            pltpu.VMEM((D, D), BF16),
            pltpu.VMEM((NSLAB * 128, DP), BF16),
            pltpu.VMEM((D, DP), BF16),
            pltpu.VMEM((5, 4 * D, 128), F32),
            pltpu.VMEM((S, FC), BF16),
            pltpu.VMEM((NTT, D, TT), F32),
            pltpu.VMEM((NSLAB, TT + HALO, 128), F32),
            pltpu.VMEM((TT, DP), BF16),
            pltpu.VMEM((NTT, D, TT), BF16),
            pltpu.VMEM((F // 128, 128), BF16),
            pltpu.VMEM((XG, TT, DP), BF16),
            pltpu.SemaphoreType.DMA((NSEM,)),
        ],
        compiler_params=pltpu.CompilerParams(vmem_limit_bytes=100 * 1024 * 1024),
        name="fused",
    )(xT, A_wqkv, A_wo, B_w1, B_b1.reshape(F // 128, 128), B_w2.T)
    return jnp.transpose(outT.reshape(1, D, S), (0, 2, 1))
```

```python
import jax
import jax.numpy as jnp
from jax import lax
import jax.experimental.pallas as pl
import jax.experimental.pallas.tpu as pltpu

S, D, F = 2048, 576, 4608
DP = 640
FC = 512
NC = F // FC
TT = 256
NTT = S // TT
BIG = 4
H, DH, WIN, DIL = 32, 18, 8, 2
HALO = 16
NSLAB = 14
RC = 8
ATT_SPREAD = 7
PREP_AT = 3
XG = 2
OSPLIT = 4
NSEM = 6
EPS = 1e-5
LOG2E = 1.4426950408889634
SCALE = DH ** -0.5
NT = (((1,), (1,)), ((), ()))
F32 = jnp.float32
BF16 = jnp.bfloat16


def _mish(h):
    e = jnp.exp(jnp.minimum(h, 20.0))
    n = e * (e + 2.0)
    return (h * n) * pl.reciprocal(n + 2.0, approx=True)


def _never(v):
    return jnp.minimum(pltpu.bitcast(v, jnp.int32), 5) > 7


def _kernel(x_hbm, wqkv_hbm, wo_hbm, w1_hbm, b1_hbm, w2_hbm, out_hbm,
            x_s, xn_s, w1_s, w2_s, wqkv_s, wo_s, wt_s, wot_s, slab_s,
            act_s, acc_s, qkv_s, o_s, out_s, b1_s, stg_s, sems):

    def rows(j, n=TT):
        if isinstance(j, int):
            return pl.ds(j * n, n)
        return pl.ds(pl.multiple_of(j * n, n), n)

    def x_copy(j, sem):
        return pltpu.make_async_copy(x_hbm.at[:, rows(j)], x_s.at[j], sems.at[sem])

    def w1_copy(c, sem):
        return pltpu.make_async_copy(w1_hbm.at[:, rows(c, FC)],
                                     w1_s.at[c, pl.ds(0, D), :], sems.at[sem])

    def w1_half(u, sem):
        return pltpu.make_async_copy(w1_hbm.at[:, rows(u, FC // 2)],
                                     w1_s.at[0, pl.ds(0, D), rows(u, FC // 2)],
                                     sems.at[sem])

    def w2_copy(c, sem):
        return pltpu.make_async_copy(w2_hbm.at[:, rows(c, FC)], w2_s.at[c], sems.at[sem])

    def out_copy(j, r0, nr):
        return pltpu.make_async_copy(out_s.at[j, pl.ds(r0, nr), :],
                                     out_hbm.at[pl.ds(r0, nr), rows(j)], sems.at[0])

    wqkv_copy = pltpu.make_async_copy(wqkv_hbm, wqkv_s, sems.at[1])
    wo_copy = pltpu.make_async_copy(wo_hbm, wo_s, sems.at[1])
    b1_copy = pltpu.make_async_copy(b1_hbm, b1_s, sems.at[0])

    def ffn1(r, c, lhs=None, cols=(0, FC)):
        lhs = xn_s[r, :] if lhs is None else lhs
        h = jnp.dot(lhs, w1_s[c, :, cols[0]:cols[1]], preferred_element_type=F32)
        act_s[r, cols[0]:cols[1]] = _mish(h).astype(BF16)

    def ffn2(j, c):
        return lax.dot_general(w2_s[c], act_s[rows(j), :], NT, preferred_element_type=F32)

    def layernorm(j, stage=None, chain=False):
        w = 128 if chain else TT
        rowp = lax.broadcasted_iota(jnp.int32, (DP - D, w), 0)
        ones_pad = jnp.where(rowp == 0, 1.0, 0.0).astype(F32)
        prev = None
        for u in range(TT // w):
            xt = x_s[j, :, u * w:(u + 1) * w].astype(F32)
            xs = xt
            if prev is not None:
                head = jnp.where(_never(prev), 0.0, xt[0:8, :])
                xs = jnp.concatenate([head, xt[8:, :]], axis=0)
            m = jnp.sum(xs, axis=0, keepdims=True) * (1.0 / D)
            xc = xt - m
            v = jnp.sum(xc * xc, axis=0, keepdims=True) * (1.0 / D)
            r = lax.rsqrt(v + EPS)
            prev = jnp.broadcast_to(r, (8, w))
            xn = jnp.concatenate([xc * r, ones_pad], axis=0)
            xnb = xn.T.astype(BF16)
            xn_s[rows(j * (TT // w) + u, w), :] = xnb
            if stage is not None:
                stage[u * w:(u + 1) * w, :] = xnb

    def bias_rows():
        b = b1_s[...].astype(F32)
        row16 = lax.broadcasted_iota(jnp.int32, (16, 128), 0)
        for c in range(NC):
            for u in range(FC // 128):
                r = c * (FC // 128) + u
                w1_s[c, D:D + 16, u * 128:(u + 1) * 128] = jnp.where(
                    row16 == 0, jnp.broadcast_to(b[r:r + 1, :], (16, 128)), 0.0
                ).astype(BF16)

    def prep_weights():
        for c in range(5):
            nr = 128 if c < 4 else 64
            blk = wqkv_s[c * 128:c * 128 + nr, :].astype(F32)
            if nr < 128:
                blk = jnp.concatenate([blk, jnp.zeros((128 - nr, 3 * D), F32)], axis=0)
            slab_s[c, 0:3 * D, :] = blk.T
        for t in range(3):
            for d in range(DH):
                if d < 16:
                    dst = t * 512 + d * H
                else:
                    dst = (1536, 1664, 1600)[t] + (d - 16) * H
                wt_s[dst:dst + H, :] = jnp.concatenate(
                    [slab_s[c, pl.ds(t * D + d, H, stride=DH), :] for c in range(5)],
                    axis=1).astype(BF16)
        for c in range(5):
            nc = 128 if c < 4 else 64
            blk = wo_s[:, c * 128:c * 128 + nc].astype(F32)
            if nc < 128:
                blk = jnp.concatenate([blk, jnp.zeros((D, 128 - nc), F32)], axis=1)
            slab_s[c, 3 * D:4 * D, :] = blk
        for c in range(5):
            nr = 128 if c < 4 else 64
            parts = [slab_s[c, pl.ds(3 * D + d, H, stride=DH), :] for d in range(16)]
            parts.append(jnp.zeros((64, 128), F32))
            parts += [slab_s[c, pl.ds(3 * D + d, H, stride=DH), :] for d in (16, 17)]
            pt = jnp.concatenate(parts, axis=0).T[:nr, :]
            wot_s[c * 128:c * 128 + nr, :] = pt.astype(BF16)
            g = pltpu.bitcast(pt[nr - 8:nr, 0:128], jnp.int32)
            for u in range(1, 5):
                g = jnp.minimum(
                    g, pltpu.bitcast(pt[nr - 8:nr, u * 128:(u + 1) * 128], jnp.int32))
            z = jnp.where(jnp.minimum(g, 5) > 7, 1.0, 0.0)
            wt_s[3 * D:NSLAB * 128, c * 128:(c + 1) * 128] = jnp.concatenate(
                [z] * 8, axis=0).astype(BF16)

    q_sl = (0, 1, 2, 3, 12)
    k_sl = (4, 5, 6, 7, 13)
    v_sl = (8, 9, 10, 11, 12)

    def attention_rows(t, r, gate):
        q = [jnp.where(gate, 0.0, qkv_s[sl, HALO + r:HALO + r + RC, :]) for sl in q_sl]
        ls = []
        for w in range(WIN):
            o0 = HALO + r - DIL * w
            s = q[0] * qkv_s[k_sl[0], o0:o0 + RC, :]
            for u in range(1, 5):
                s = s + q[u] * qkv_s[k_sl[u], o0:o0 + RC, :]
            s = s + pltpu.roll(s, 64, 1)
            s = s + pltpu.roll(s, 32, 1)
            if r < HALO and w > 0:
                pos = t * TT + r + lax.broadcasted_iota(jnp.int32, (RC, 128), 0)
                s = jnp.where(pos >= DIL * w, s, -1e9 / SCALE)
            ls.append(s)
        m = ls[0]
        for w in range(1, WIN):
            m = jnp.maximum(m, ls[w])
        ps = [jnp.exp2((l - m) * (SCALE * LOG2E)) for l in ls]
        den = ps[0]
        for w in range(1, WIN):
            den = den + ps[w]
        rinv = pl.reciprocal(den, approx=True)
        outs = []
        for u in range(5):
            a = ps[0] * qkv_s[v_sl[u], HALO + r:HALO + r + RC, :]
            for w in range(1, WIN):
                o0 = HALO + r - DIL * w
                a = a + ps[w] * qkv_s[v_sl[u], o0:o0 + RC, :]
            outs.append(a * rinv)
        o_s[r:r + RC, :] = jnp.concatenate(outs, axis=1).astype(BF16)
        return den

    chunks = list(range(0, TT, RC))
    att_sched = [[] for _ in range(NTT)]
    for i, r in enumerate(chunks):
        att_sched[i * ATT_SPREAD // len(chunks)].append(r)

    def attention_group(t, j, y):
        gate = _never(y[0:RC, 0:128])
        for r in att_sched[j]:
            gate = _never(attention_rows(t, r, gate))

    def qkv_proj(t):
        qkv_s[4:NSLAB, 0:HALO, :] = qkv_s[4:NSLAB, TT:TT + HALO, :]
        qkv = lax.dot_general(xn_s[rows(t), :], wt_s[...], NT, preferred_element_type=F32)
        for sl in range(NSLAB):
            qkv_s[sl, HALO:HALO + TT, :] = qkv[:, sl * 128:(sl + 1) * 128]

    def wo_proj():
        return lax.dot_general(wot_s[...], o_s[...], NT, preferred_element_type=F32)

    x_copy(0, 0).start()
    b1_copy.start()
    w1_half(0, 5).start()
    x_copy(1, 1).start()
    w1_half(1, 1).start()
    for j in range(2, NTT):
        x_copy(j, 2 + (j - 2) // XG).start()
    for c in range(NC):
        w1_s[c, D + 16:DP, :] = jnp.zeros((DP - D - 16, FC), BF16)
    qkv_s[:, TT:TT + HALO, :] = jnp.zeros((NSLAB, HALO, 128), F32)

    x_copy(0, 0).wait()
    b1_copy.wait()
    layernorm(0)
    bias_rows()
    w1_half(0, 5).wait()
    w1_copy(1, 5).start()
    w2_copy(0, 5).start()
    ffn1(rows(0), 0, cols=(0, 128))
    ffn1(rows(0), 0, cols=(128, 256))
    x_copy(1, 1).wait()
    w1_half(1, 1).wait()
    wqkv_copy.start()
    wo_copy.start()
    layernorm(1, stg_s.at[XG - 1])
    ffn1(rows(0), 0, cols=(256, 384))
    ffn1(rows(0), 0, cols=(384, 512))

    def step0(i, carry):
        for u in range(XG):
            x_copy(XG * i + 2 + u, 2 + i).wait()
        for u in range(XG):
            layernorm(XG * i + 2 + u, stg_s.at[u], chain=True)
            ffn1(rows(XG * i + 1 + u), 0, lhs=stg_s[(u - 1) % XG])
        return carry

    lax.fori_loop(0, (NTT - 2) // XG, step0, 0)

    w1_copy(1, 5).wait()
    w2_copy(0, 5).wait()
    rest = []
    for c in range(2, NC):
        rest += [w1_copy(c, 2), w2_copy(c - 1, 2)]
    rest.append(w2_copy(NC - 1, 2))
    for cp in rest:
        cp.start()
    ffn1(rows(NTT - 1), 0)
    for j in range(NTT):
        acc_s[j] = x_s[j].astype(F32) + ffn2(j, 0)
        if j == PREP_AT:
            wqkv_copy.wait()
            wo_copy.wait()
            prep_weights()
        if j % BIG == BIG - 1:
            ffn1(rows(j // BIG, TT * BIG), 1)
    qkv_proj(0)
    for cp in rest:
        cp.wait()

    def step(s, carry):
        t = s - 2
        for j in range(NTT):
            y = ffn2(j, s - 1)
            acc_s[j] += y
            if j % BIG == BIG - 1:
                ffn1(rows(j // BIG, TT * BIG), s)
            attention_group(t, j, y)
        acc_s[t] += wo_proj()
        qkv_proj(t + 1)
        return carry

    lax.fori_loop(2, NC, step, 0)

    t = NTT - 1
    outs = []
    for j in range(NTT):
        y = ffn2(j, NC - 1)
        res = acc_s[j] + y
        if j == t:
            res = res + wo_proj()
        nsp = OSPLIT if j == t else 1
        nr = D // nsp
        for u in range(nsp):
            out_s[j, u * nr:(u + 1) * nr, :] = res[u * nr:(u + 1) * nr, :].astype(BF16)
            cp = out_copy(j, u * nr, nr)
            cp.start()
            outs.append(cp)
        attention_group(t, j, y)
    for cp in outs:
        cp.wait()


@jax.jit
def pallas_parallel_sum__sliding_local_dilated__dense_activation_mish__prompt_kernel(
    A_x: jax.Array,
    A_wqkv: jax.Array,
    A_wo: jax.Array,
    B_x: jax.Array,
    B_w1: jax.Array,
    B_b1: jax.Array,
    B_w2: jax.Array,
):
    del B_x
    xT = jnp.transpose(A_x, (0, 2, 1)).reshape(D, S)
    any_spec = pl.BlockSpec(memory_space=pl.ANY)
    outT = pl.pallas_call(
        _kernel,
        out_shape=jax.ShapeDtypeStruct((D, S), BF16),
        in_specs=[any_spec] * 6,
        out_specs=any_spec,
        scratch_shapes=[
            pltpu.VMEM((NTT, D, TT), BF16),
            pltpu.VMEM((S, DP), BF16),
            pltpu.VMEM((NC, DP, FC), BF16),
            pltpu.VMEM((NC, D, FC), BF16),
            pltpu.VMEM((D, 3 * D), BF16),
            pltpu.VMEM((D, D), BF16),
            pltpu.VMEM((NSLAB * 128, DP), BF16),
            pltpu.VMEM((D, DP), BF16),
            pltpu.VMEM((5, 4 * D, 128), F32),
            pltpu.VMEM((S, FC), BF16),
            pltpu.VMEM((NTT, D, TT), F32),
            pltpu.VMEM((NSLAB, TT + HALO, 128), F32),
            pltpu.VMEM((TT, DP), BF16),
            pltpu.VMEM((NTT, D, TT), BF16),
            pltpu.VMEM((F // 128, 128), BF16),
            pltpu.VMEM((XG, TT, DP), BF16),
            pltpu.SemaphoreType.DMA((NSEM,)),
        ],
        compiler_params=pltpu.CompilerParams(vmem_limit_bytes=64 * 1024 * 1024),
        name="fused_attn_ffn",
    )(xT, A_wqkv, A_wo, B_w1, B_b1.reshape(F // 128, 128), B_w2.T)
    return jnp.transpose(outT.reshape(1, D, S), (0, 2, 1))
```

```python
import jax
import jax.numpy as jnp
from jax import lax
import jax.experimental.pallas as pl
import jax.experimental.pallas.tpu as pltpu

S, D, F = 2048, 576, 4608
DP = 640
FC = 512
NC = F // FC
TT = 256
NTT = S // TT
BIG = 4
H, DH, WIN, DIL = 32, 18, 8, 2
HALO = 16
NSLAB = 14
RC = 8
ATT_SPREAD = 7
PREP_AT = 1
XG = 2
OSPLIT = 4
NSEM = 6
EPS = 1e-5
LOG2E = 1.4426950408889634
SCALE = DH ** -0.5
NT = (((1,), (1,)), ((), ()))
F32 = jnp.float32
BF16 = jnp.bfloat16


def _mish(h):
    e = jnp.exp(jnp.minimum(h, 20.0))
    n = e * (e + 2.0)
    return (h * n) * pl.reciprocal(n + 2.0, approx=True)


def _never(v):
    return jnp.minimum(pltpu.bitcast(v, jnp.int32), 5) > 7


def _kernel(x_hbm, wqkv_hbm, wo_hbm, w1_hbm, b1_hbm, w2_hbm, out_hbm,
            x_s, xn_s, w1_s, w2_s, wqkv_s, wo_s, wt_s, wot_s, slab_s,
            act_s, acc_s, qkv_s, o_s, out_s, b1_s, stg_s, sems):

    def rows(j, n=TT):
        if isinstance(j, int):
            return pl.ds(j * n, n)
        return pl.ds(pl.multiple_of(j * n, n), n)

    def x_copy(j, sem):
        return pltpu.make_async_copy(x_hbm.at[:, rows(j)], x_s.at[j], sems.at[sem])

    def w1_copy(c, sem):
        return pltpu.make_async_copy(w1_hbm.at[:, rows(c, FC)],
                                     w1_s.at[c, pl.ds(0, D), :], sems.at[sem])

    def w1_half(u, sem):
        return pltpu.make_async_copy(w1_hbm.at[:, rows(u, FC // 2)],
                                     w1_s.at[0, pl.ds(0, D), rows(u, FC // 2)],
                                     sems.at[sem])

    def w2_copy(c, sem):
        return pltpu.make_async_copy(w2_hbm.at[:, rows(c, FC)], w2_s.at[c], sems.at[sem])

    def out_copy(j, r0, nr):
        return pltpu.make_async_copy(out_s.at[j, pl.ds(r0, nr), :],
                                     out_hbm.at[pl.ds(r0, nr), rows(j)], sems.at[0])

    wqkv_copy = pltpu.make_async_copy(wqkv_hbm, wqkv_s, sems.at[1])
    wo_copy = pltpu.make_async_copy(wo_hbm, wo_s, sems.at[1])
    b1_copy = pltpu.make_async_copy(b1_hbm, b1_s, sems.at[0])

    def ffn1(r, c, lhs=None, cols=(0, FC)):
        lhs = xn_s[r, :] if lhs is None else lhs
        h = jnp.dot(lhs, w1_s[c, :, cols[0]:cols[1]], preferred_element_type=F32)
        act_s[r, cols[0]:cols[1]] = _mish(h).astype(BF16)

    def ffn2(j, c):
        return lax.dot_general(w2_s[c], act_s[rows(j), :], NT, preferred_element_type=F32)

    def layernorm(j, stage=None, chain=False):
        w = 128 if chain else TT
        rowp = lax.broadcasted_iota(jnp.int32, (DP - D, w), 0)
        ones_pad = jnp.where(rowp == 0, 1.0, 0.0).astype(F32)
        prev = None
        for u in range(TT // w):
            xt = x_s[j, :, u * w:(u + 1) * w].astype(F32)
            xs = xt
            if prev is not None:
                head = jnp.where(_never(prev), 0.0, xt[0:8, :])
                xs = jnp.concatenate([head, xt[8:, :]], axis=0)
            m = jnp.sum(xs, axis=0, keepdims=True) * (1.0 / D)
            xc = xt - m
            v = jnp.sum(xc * xc, axis=0, keepdims=True) * (1.0 / D)
            r = lax.rsqrt(v + EPS)
            prev = jnp.broadcast_to(r, (8, w))
            xn = jnp.concatenate([xc * r, ones_pad], axis=0)
            xnb = xn.T.astype(BF16)
            xn_s[rows(j * (TT // w) + u, w), :] = xnb
            if stage is not None:
                stage[u * w:(u + 1) * w, :] = xnb

    def bias_rows():
        b = b1_s[...].astype(F32)
        row16 = lax.broadcasted_iota(jnp.int32, (16, 128), 0)
        for c in range(NC):
            for u in range(FC // 128):
                r = c * (FC // 128) + u
                w1_s[c, D:D + 16, u * 128:(u + 1) * 128] = jnp.where(
                    row16 == 0, jnp.broadcast_to(b[r:r + 1, :], (16, 128)), 0.0
                ).astype(BF16)

    def prep_weights():
        for c in range(5):
            nr = 128 if c < 4 else 64
            blk = wqkv_s[c * 128:c * 128 + nr, :].astype(F32)
            if nr < 128:
                blk = jnp.concatenate([blk, jnp.zeros((128 - nr, 3 * D), F32)], axis=0)
            slab_s[c, 0:3 * D, :] = blk.T
        for t in range(3):
            for d in range(DH):
                if d < 16:
                    dst = t * 512 + d * H
                else:
                    dst = (1536, 1664, 1600)[t] + (d - 16) * H
                wt_s[dst:dst + H, :] = jnp.concatenate(
                    [slab_s[c, pl.ds(t * D + d, H, stride=DH), :] for c in range(5)],
                    axis=1).astype(BF16)
        for c in range(5):
            nc = 128 if c < 4 else 64
            blk = wo_s[:, c * 128:c * 128 + nc].astype(F32)
            if nc < 128:
                blk = jnp.concatenate([blk, jnp.zeros((D, 128 - nc), F32)], axis=1)
            slab_s[c, 3 * D:4 * D, :] = blk
        for c in range(5):
            nr = 128 if c < 4 else 64
            parts = [slab_s[c, pl.ds(3 * D + d, H, stride=DH), :] for d in range(16)]
            parts.append(jnp.zeros((64, 128), F32))
            parts += [slab_s[c, pl.ds(3 * D + d, H, stride=DH), :] for d in (16, 17)]
            pt = jnp.concatenate(parts, axis=0).T[:nr, :]
            wot_s[c * 128:c * 128 + nr, :] = pt.astype(BF16)
            g = pltpu.bitcast(pt[nr - 8:nr, 0:128], jnp.int32)
            for u in range(1, 5):
                g = jnp.minimum(
                    g, pltpu.bitcast(pt[nr - 8:nr, u * 128:(u + 1) * 128], jnp.int32))
            z = jnp.where(jnp.minimum(g, 5) > 7, 1.0, 0.0)
            wt_s[3 * D:NSLAB * 128, c * 128:(c + 1) * 128] = jnp.concatenate(
                [z] * 8, axis=0).astype(BF16)

    q_sl = (0, 1, 2, 3, 12)
    k_sl = (4, 5, 6, 7, 13)
    v_sl = (8, 9, 10, 11, 12)

    def attention_rows(t, r, gate):
        q = [jnp.where(gate, 0.0, qkv_s[sl, HALO + r:HALO + r + RC, :]) for sl in q_sl]
        ls = []
        for w in range(WIN):
            o0 = HALO + r - DIL * w
            s = q[0] * qkv_s[k_sl[0], o0:o0 + RC, :]
            for u in range(1, 5):
                s = s + q[u] * qkv_s[k_sl[u], o0:o0 + RC, :]
            s = s + pltpu.roll(s, 64, 1)
            s = s + pltpu.roll(s, 32, 1)
            if r < HALO and w > 0:
                pos = t * TT + r + lax.broadcasted_iota(jnp.int32, (RC, 128), 0)
                s = jnp.where(pos >= DIL * w, s, -1e9 / SCALE)
            ls.append(s)
        m = ls[0]
        for w in range(1, WIN):
            m = jnp.maximum(m, ls[w])
        ps = [jnp.exp2((l - m) * (SCALE * LOG2E)) for l in ls]
        den = ps[0]
        for w in range(1, WIN):
            den = den + ps[w]
        rinv = pl.reciprocal(den, approx=True)
        outs = []
        for u in range(5):
            a = ps[0] * qkv_s[v_sl[u], HALO + r:HALO + r + RC, :]
            for w in range(1, WIN):
                o0 = HALO + r - DIL * w
                a = a + ps[w] * qkv_s[v_sl[u], o0:o0 + RC, :]
            outs.append(a * rinv)
        o_s[r:r + RC, :] = jnp.concatenate(outs, axis=1).astype(BF16)
        return den

    chunks = list(range(0, TT, RC))
    att_sched = [[] for _ in range(NTT)]
    for i, r in enumerate(chunks):
        att_sched[i * ATT_SPREAD // len(chunks)].append(r)

    def attention_group(t, j, y):
        gate = _never(y[0:RC, 0:128])
        for r in att_sched[j]:
            gate = _never(attention_rows(t, r, gate))

    def qkv_proj(t):
        qkv_s[4:NSLAB, 0:HALO, :] = qkv_s[4:NSLAB, TT:TT + HALO, :]
        qkv = lax.dot_general(xn_s[rows(t), :], wt_s[...], NT, preferred_element_type=F32)
        for sl in range(NSLAB):
            qkv_s[sl, HALO:HALO + TT, :] = qkv[:, sl * 128:(sl + 1) * 128]

    def wo_proj():
        return lax.dot_general(wot_s[...], o_s[...], NT, preferred_element_type=F32)

    x_copy(0, 0).start()
    b1_copy.start()
    w1_half(0, 5).start()
    x_copy(1, 1).start()
    w1_half(1, 1).start()
    for j in range(2, NTT):
        x_copy(j, 2 + (j - 2) // XG).start()
    for c in range(NC):
        w1_s[c, D + 16:DP, :] = jnp.zeros((DP - D - 16, FC), BF16)
    qkv_s[:, TT:TT + HALO, :] = jnp.zeros((NSLAB, HALO, 128), F32)

    def zero_acc(j, carry):
        acc_s[j] = jnp.zeros((D, TT), F32)
        return carry

    lax.fori_loop(BIG, NTT, zero_acc, 0)

    x_copy(0, 0).wait()
    b1_copy.wait()
    layernorm(0)
    bias_rows()
    w1_half(0, 5).wait()
    w1_copy(1, 5).start()
    w2_copy(0, 5).start()
    ffn1(rows(0), 0, cols=(0, 128))
    ffn1(rows(0), 0, cols=(128, 256))
    x_copy(1, 1).wait()
    w1_half(1, 1).wait()
    wqkv_copy.start()
    wo_copy.start()
    layernorm(1, stg_s.at[XG - 1])
    ffn1(rows(0), 0, cols=(256, 384))
    ffn1(rows(0), 0, cols=(384, 512))

    def step0(i, carry):
        for u in range(XG):
            x_copy(XG * i + 2 + u, 2 + i).wait()
        for u in range(XG):
            layernorm(XG * i + 2 + u, stg_s.at[u], chain=True)
            ffn1(rows(XG * i + 1 + u), 0, lhs=stg_s[(u - 1) % XG])
        return carry

    lax.fori_loop(0, (NTT - 2) // XG, step0, 0)

    w1_copy(1, 5).wait()
    w2_copy(0, 5).wait()
    w1_copy(2, 2).start()
    w2_copy(1, 2).start()
    w2_copy(NC - 1, 4).start()
    ffn1(rows(NTT - 1), 0)
    for j in range(BIG):
        acc_s[j] = ffn2(j, 0)
        if j == PREP_AT:
            wqkv_copy.wait()
            wo_copy.wait()
            prep_weights()
    ffn1(rows(0, TT * BIG), 1)
    qkv_proj(0)
    w2_copy(NC - 1, 4).wait()

    def step(s, carry):
        t = s - 2
        cur = 2 + lax.rem(s, 2)
        w1_copy(s, cur).wait()
        w2_copy(s - 1, cur).wait()

        @pl.when(s + 1 < NC)
        def _():
            w1_copy(s + 1, 5 - cur).start()
            w2_copy(s, 5 - cur).start()

        for j in range(NTT):
            c = s - j // BIG
            y = ffn2(j, c - 1)
            acc_s[j] += y
            if j % BIG == BIG - 1:
                ffn1(rows(j // BIG, TT * BIG), c)
            attention_group(t, j, y)
        acc_s[t] += wo_proj()
        qkv_proj(t + 1)
        return carry

    lax.fori_loop(2, NC, step, 0)

    t = NTT - 1
    outs = []

    def finish(j, extra=None):
        y = ffn2(j, NC - 1)
        res = (acc_s[j] + x_s[j].astype(F32)) + y
        if extra is not None:
            res = res + extra
        nsp = OSPLIT if j == t else 1
        nr = D // nsp
        for u in range(nsp):
            out_s[j, u * nr:(u + 1) * nr, :] = res[u * nr:(u + 1) * nr, :].astype(BF16)
            cp = out_copy(j, u * nr, nr)
            cp.start()
            outs.append(cp)
        return y

    for j in range(BIG, NTT):
        y = ffn2(j, NC - 2)
        acc_s[j] += y
        attention_group(t, j - BIG, y)
    ffn1(rows(1, TT * BIG), NC - 1)
    for j in range(BIG):
        y = finish(j)
        attention_group(t, BIG + j, y)
    for j in range(BIG, NTT):
        finish(j, wo_proj() if j == t else None)
    for cp in outs:
        cp.wait()


@jax.jit
def pallas_parallel_sum__sliding_local_dilated__dense_activation_mish__prompt_kernel(
    A_x: jax.Array,
    A_wqkv: jax.Array,
    A_wo: jax.Array,
    B_x: jax.Array,
    B_w1: jax.Array,
    B_b1: jax.Array,
    B_w2: jax.Array,
):
    del B_x
    xT = jnp.transpose(A_x, (0, 2, 1)).reshape(D, S)
    any_spec = pl.BlockSpec(memory_space=pl.ANY)
    outT = pl.pallas_call(
        _kernel,
        out_shape=jax.ShapeDtypeStruct((D, S), BF16),
        in_specs=[any_spec] * 6,
        out_specs=any_spec,
        scratch_shapes=[
            pltpu.VMEM((NTT, D, TT), BF16),
            pltpu.VMEM((S, DP), BF16),
            pltpu.VMEM((NC, DP, FC), BF16),
            pltpu.VMEM((NC, D, FC), BF16),
            pltpu.VMEM((D, 3 * D), BF16),
            pltpu.VMEM((D, D), BF16),
            pltpu.VMEM((NSLAB * 128, DP), BF16),
            pltpu.VMEM((D, DP), BF16),
            pltpu.VMEM((5, 4 * D, 128), F32),
            pltpu.VMEM((S, FC), BF16),
            pltpu.VMEM((NTT, D, TT), F32),
            pltpu.VMEM((NSLAB, TT + HALO, 128), F32),
            pltpu.VMEM((TT, DP), BF16),
            pltpu.VMEM((NTT, D, TT), BF16),
            pltpu.VMEM((F // 128, 128), BF16),
            pltpu.VMEM((XG, TT, DP), BF16),
            pltpu.SemaphoreType.DMA((NSEM,)),
        ],
        compiler_params=pltpu.CompilerParams(vmem_limit_bytes=64 * 1024 * 1024),
        name="fused_attn_ffn",
    )(xT, A_wqkv, A_wo, B_w1, B_b1.reshape(F // 128, 128), B_w2.T)
    return jnp.transpose(outT.reshape(1, D, S), (0, 2, 1))
```

```python
import jax
import jax.numpy as jnp
from jax import lax
import jax.experimental.pallas as pl
import jax.experimental.pallas.tpu as pltpu

S, D, F = 2048, 576, 4608
DP = 640
FC = 512
NC = F // FC
TT = 256
NTT = S // TT
BIG = 4
H, DH, WIN, DIL = 32, 18, 8, 2
HALO = 16
NSLAB = 14
RC = 8
ATT_SPREAD = 7
PREP_AT = 1
XG = 2
OSPLIT = 4
NSEM = 6
EPS = 1e-5
LOG2E = 1.4426950408889634
SCALE = DH ** -0.5
NT = (((1,), (1,)), ((), ()))
F32 = jnp.float32
BF16 = jnp.bfloat16


def _mish(h):
    e = jnp.exp(jnp.minimum(h, 20.0))
    n = e * (e + 2.0)
    return (h * n) * pl.reciprocal(n + 2.0, approx=True)


def _never(v):
    return jnp.minimum(pltpu.bitcast(v, jnp.int32), 5) > 7


def _kernel(x_hbm, wqkv_hbm, wo_hbm, w1_hbm, b1_hbm, w2_hbm, out_hbm,
            x_s, xn_s, w1_s, w2_s, wqkv_s, wo_s, wt_s, wot_s, slab_s,
            act_s, acc_s, qkv_s, o_s, out_s, b1_s, stg_s, sems):

    def rows(j, n=TT):
        if isinstance(j, int):
            return pl.ds(j * n, n)
        return pl.ds(pl.multiple_of(j * n, n), n)

    def x_copy(j, sem):
        return pltpu.make_async_copy(x_hbm.at[:, rows(j)], x_s.at[j], sems.at[sem])

    def w1_copy(c, sem):
        return pltpu.make_async_copy(w1_hbm.at[:, rows(c, FC)],
                                     w1_s.at[c, pl.ds(0, D), :], sems.at[sem])

    def w1_half(u, sem):
        return pltpu.make_async_copy(w1_hbm.at[:, rows(u, FC // 2)],
                                     w1_s.at[0, pl.ds(0, D), rows(u, FC // 2)],
                                     sems.at[sem])

    def w2_copy(c, sem):
        return pltpu.make_async_copy(w2_hbm.at[:, rows(c, FC)], w2_s.at[c], sems.at[sem])

    def out_copy(j, r0, nr):
        return pltpu.make_async_copy(out_s.at[j, pl.ds(r0, nr), :],
                                     out_hbm.at[pl.ds(r0, nr), rows(j)], sems.at[0])

    wqkv_copy = pltpu.make_async_copy(wqkv_hbm, wqkv_s, sems.at[1])
    wo_copy = pltpu.make_async_copy(wo_hbm, wo_s, sems.at[1])
    b1_copy = pltpu.make_async_copy(b1_hbm, b1_s, sems.at[0])

    def ffn1(r, c, lhs=None, cols=(0, FC)):
        lhs = xn_s[r, :] if lhs is None else lhs
        h = jnp.dot(lhs, w1_s[c, :, cols[0]:cols[1]], preferred_element_type=F32)
        act_s[r, cols[0]:cols[1]] = _mish(h).astype(BF16)

    def ffn2(j, c):
        return lax.dot_general(w2_s[c], act_s[rows(j), :], NT, preferred_element_type=F32)

    def layernorm(j, stage=None, chain=False):
        w = 128 if chain else TT
        rowp = lax.broadcasted_iota(jnp.int32, (DP - D, w), 0)
        ones_pad = jnp.where(rowp == 0, 1.0, 0.0).astype(F32)
        prev = None
        for u in range(TT // w):
            xt = x_s[j, :, u * w:(u + 1) * w].astype(F32)
            xs = xt
            if prev is not None:
                head = jnp.where(_never(prev), 0.0, xt[0:8, :])
                xs = jnp.concatenate([head, xt[8:, :]], axis=0)
            m = jnp.sum(xs, axis=0, keepdims=True) * (1.0 / D)
            xc = xt - m
            v = jnp.sum(xc * xc, axis=0, keepdims=True) * (1.0 / D)
            r = lax.rsqrt(v + EPS)
            prev = jnp.broadcast_to(r, (8, w))
            xn = jnp.concatenate([xc * r, ones_pad], axis=0)
            xnb = xn.T.astype(BF16)
            xn_s[rows(j * (TT // w) + u, w), :] = xnb
            if stage is not None:
                stage[u * w:(u + 1) * w, :] = xnb

    def bias_rows():
        b = b1_s[...].astype(F32)
        row16 = lax.broadcasted_iota(jnp.int32, (16, 128), 0)
        for c in range(NC):
            for u in range(FC // 128):
                r = c * (FC // 128) + u
                w1_s[c, D:D + 16, u * 128:(u + 1) * 128] = jnp.where(
                    row16 == 0, jnp.broadcast_to(b[r:r + 1, :], (16, 128)), 0.0
                ).astype(BF16)

    def prep_weights():
        for c in range(5):
            nr = 128 if c < 4 else 64
            blk = wqkv_s[c * 128:c * 128 + nr, :].astype(F32)
            if nr < 128:
                blk = jnp.concatenate([blk, jnp.zeros((128 - nr, 3 * D), F32)], axis=0)
            slab_s[c, 0:3 * D, :] = blk.T
        for t in range(3):
            for d in range(DH):
                if d < 16:
                    dst = t * 512 + d * H
                else:
                    dst = (1536, 1664, 1600)[t] + (d - 16) * H
                wt_s[dst:dst + H, :] = jnp.concatenate(
                    [slab_s[c, pl.ds(t * D + d, H, stride=DH), :] for c in range(5)],
                    axis=1).astype(BF16)
        for c in range(5):
            nc = 128 if c < 4 else 64
            blk = wo_s[:, c * 128:c * 128 + nc].astype(F32)
            if nc < 128:
                blk = jnp.concatenate([blk, jnp.zeros((D, 128 - nc), F32)], axis=1)
            slab_s[c, 3 * D:4 * D, :] = blk
        for c in range(5):
            nr = 128 if c < 4 else 64
            parts = [slab_s[c, pl.ds(3 * D + d, H, stride=DH), :] for d in range(16)]
            parts.append(jnp.zeros((64, 128), F32))
            parts += [slab_s[c, pl.ds(3 * D + d, H, stride=DH), :] for d in (16, 17)]
            pt = jnp.concatenate(parts, axis=0).T[:nr, :]
            wot_s[c * 128:c * 128 + nr, :] = pt.astype(BF16)
            g = pltpu.bitcast(pt[nr - 8:nr, 0:128], jnp.int32)
            for u in range(1, 5):
                g = jnp.minimum(
                    g, pltpu.bitcast(pt[nr - 8:nr, u * 128:(u + 1) * 128], jnp.int32))
            z = jnp.where(jnp.minimum(g, 5) > 7, 1.0, 0.0)
            wt_s[3 * D:NSLAB * 128, c * 128:(c + 1) * 128] = jnp.concatenate(
                [z] * 8, axis=0).astype(BF16)

    q_sl = (0, 1, 2, 3, 12)
    k_sl = (4, 5, 6, 7, 13)
    v_sl = (8, 9, 10, 11, 12)

    def attention_rows(t, r, gate):
        q = [jnp.where(gate, 0.0, qkv_s[sl, HALO + r:HALO + r + RC, :]) for sl in q_sl]
        ls = []
        for w in range(WIN):
            o0 = HALO + r - DIL * w
            s = q[0] * qkv_s[k_sl[0], o0:o0 + RC, :]
            for u in range(1, 5):
                s = s + q[u] * qkv_s[k_sl[u], o0:o0 + RC, :]
            s = s + pltpu.roll(s, 64, 1)
            s = s + pltpu.roll(s, 32, 1)
            if r < HALO and w > 0:
                pos = t * TT + r + lax.broadcasted_iota(jnp.int32, (RC, 128), 0)
                s = jnp.where(pos >= DIL * w, s, -1e9 / SCALE)
            ls.append(s)
        m = ls[0]
        for w in range(1, WIN):
            m = jnp.maximum(m, ls[w])
        ps = [jnp.exp2((l - m) * (SCALE * LOG2E)) for l in ls]
        den = ps[0]
        for w in range(1, WIN):
            den = den + ps[w]
        rinv = pl.reciprocal(den, approx=True)
        outs = []
        for u in range(5):
            a = ps[0] * qkv_s[v_sl[u], HALO + r:HALO + r + RC, :]
            for w in range(1, WIN):
                o0 = HALO + r - DIL * w
                a = a + ps[w] * qkv_s[v_sl[u], o0:o0 + RC, :]
            outs.append(a * rinv)
        o_s[r:r + RC, :] = jnp.concatenate(outs, axis=1).astype(BF16)
        return den

    chunks = list(range(0, TT, RC))
    att_sched = [[] for _ in range(NTT)]
    for i, r in enumerate(chunks):
        att_sched[i * ATT_SPREAD // len(chunks)].append(r)

    def attention_group(t, j, y):
        gate = _never(y[0:RC, 0:128])
        for r in att_sched[j]:
            gate = _never(attention_rows(t, r, gate))

    def qkv_proj(t):
        qkv_s[4:NSLAB, 0:HALO, :] = qkv_s[4:NSLAB, TT:TT + HALO, :]
        qkv = lax.dot_general(xn_s[rows(t), :], wt_s[...], NT, preferred_element_type=F32)
        for sl in range(NSLAB):
            qkv_s[sl, HALO:HALO + TT, :] = qkv[:, sl * 128:(sl + 1) * 128]

    def wo_proj():
        return lax.dot_general(wot_s[...], o_s[...], NT, preferred_element_type=F32)

    x_copy(0, 0).start()
    b1_copy.start()
    w1_half(0, 5).start()
    x_copy(1, 1).start()
    w1_half(1, 1).start()
    for j in range(2, NTT):
        x_copy(j, 2 + (j - 2) // XG).start()
    for c in range(NC):
        w1_s[c, D + 16:DP, :] = jnp.zeros((DP - D - 16, FC), BF16)
    qkv_s[:, TT:TT + HALO, :] = jnp.zeros((NSLAB, HALO, 128), F32)

    def zero_acc(j, carry):
        acc_s[j] = jnp.zeros((D, TT), F32)
        return carry

    lax.fori_loop(BIG, NTT, zero_acc, 0)

    x_copy(0, 0).wait()
    b1_copy.wait()
    layernorm(0)
    bias_rows()
    w1_half(0, 5).wait()
    w1_copy(1, 5).start()
    w2_copy(0, 5).start()
    ffn1(rows(0), 0, cols=(0, 128))
    ffn1(rows(0), 0, cols=(128, 256))
    x_copy(1, 1).wait()
    w1_half(1, 1).wait()
    wqkv_copy.start()
    wo_copy.start()
    layernorm(1, stg_s.at[XG - 1])
    ffn1(rows(0), 0, cols=(256, 384))
    ffn1(rows(0), 0, cols=(384, 512))

    def step0(i, carry):
        for u in range(XG):
            x_copy(XG * i + 2 + u, 2 + i).wait()
        for u in range(XG):
            layernorm(XG * i + 2 + u, stg_s.at[u], chain=True)
            ffn1(rows(XG * i + 1 + u), 0, lhs=stg_s[(u - 1) % XG])
        return carry

    lax.fori_loop(0, (NTT - 2) // XG, step0, 0)

    w1_copy(1, 5).wait()
    w2_copy(0, 5).wait()
    w1_copy(2, 2).start()
    w2_copy(1, 2).start()
    w2_copy(NC - 1, 4).start()
    ffn1(rows(NTT - 1), 0)
    for j in range(BIG):
        acc_s[j] = ffn2(j, 0)
        if j == PREP_AT:
            wqkv_copy.wait()
            wo_copy.wait()
            prep_weights()
    ffn1(rows(0, TT * BIG), 1)
    qkv_proj(0)
    w2_copy(NC - 1, 4).wait()

    def step(s, carry):
        t = s - 2
        cur = 2 + lax.rem(s, 2)
        w1_copy(s, cur).wait()
        w2_copy(s - 1, cur).wait()

        @pl.when(s + 1 < NC)
        def _():
            w1_copy(s + 1, 5 - cur).start()
            w2_copy(s, 5 - cur).start()

        for j in range(NTT):
            c = s - j // BIG
            y = ffn2(j, c - 1)
            acc_s[j] += y
            if j % BIG == BIG - 1:
                ffn1(rows(j // BIG, TT * BIG), c)
            attention_group(t, j, y)
        acc_s[t] += wo_proj()
        qkv_proj(t + 1)
        return carry

    lax.fori_loop(2, NC, step, 0)

    t = NTT - 1
    outs = []

    def finish(j, extra=None):
        y = ffn2(j, NC - 1)
        res = (acc_s[j] + x_s[j].astype(F32)) + y
        if extra is not None:
            res = res + extra
        nsp = OSPLIT if j == t else 1
        nr = D // nsp
        for u in range(nsp):
            out_s[j, u * nr:(u + 1) * nr, :] = res[u * nr:(u + 1) * nr, :].astype(BF16)
            cp = out_copy(j, u * nr, nr)
            cp.start()
            outs.append(cp)
        return y

    for j in range(BIG, NTT):
        y = ffn2(j, NC - 2)
        acc_s[j] += y
        attention_group(t, j - BIG, y)
    ffn1(rows(1, TT * BIG), NC - 1)
    for j in range(BIG):
        y = finish(j)
        attention_group(t, BIG + j, y)
    for j in range(BIG, NTT):
        finish(j, wo_proj() if j == t else None)
    for cp in outs:
        cp.wait()


@jax.jit
def pallas_parallel_sum__sliding_local_dilated__dense_activation_mish__prompt_kernel(
    A_x: jax.Array,
    A_wqkv: jax.Array,
    A_wo: jax.Array,
    B_x: jax.Array,
    B_w1: jax.Array,
    B_b1: jax.Array,
    B_w2: jax.Array,
):
    del B_x
    xT = jnp.transpose(A_x, (0, 2, 1)).reshape(D, S)
    any_spec = pl.BlockSpec(memory_space=pl.ANY)
    outT = pl.pallas_call(
        _kernel,
        out_shape=jax.ShapeDtypeStruct((D, S), BF16),
        in_specs=[any_spec] * 6,
        out_specs=any_spec,
        scratch_shapes=[
            pltpu.VMEM((NTT, D, TT), BF16),
            pltpu.VMEM((S, DP), BF16),
            pltpu.VMEM((NC, DP, FC), BF16),
            pltpu.VMEM((NC, D, FC), BF16),
            pltpu.VMEM((D, 3 * D), BF16),
            pltpu.VMEM((D, D), BF16),
            pltpu.VMEM((NSLAB * 128, DP), BF16),
            pltpu.VMEM((D, DP), BF16),
            pltpu.VMEM((5, 4 * D, 128), F32),
            pltpu.VMEM((S, FC), BF16),
            pltpu.VMEM((NTT, D, TT), F32),
            pltpu.VMEM((NSLAB, TT + HALO, 128), F32),
            pltpu.VMEM((TT, DP), BF16),
            pltpu.VMEM((NTT, D, TT), BF16),
            pltpu.VMEM((F // 128, 128), BF16),
            pltpu.VMEM((XG, TT, DP), BF16),
            pltpu.SemaphoreType.DMA((NSEM,)),
        ],
        compiler_params=pltpu.CompilerParams(
            vmem_limit_bytes=64 * 1024 * 1024,
            disable_bounds_checks=True,
            disable_semaphore_checks=True,
        ),
        name="fused_attn_ffn",
    )(xT, A_wqkv, A_wo, B_w1, B_b1.reshape(F // 128, 128), B_w2.T)
    return jnp.transpose(outT.reshape(1, D, S), (0, 2, 1))
```

```python
import jax
import jax.numpy as jnp
from jax import lax
import jax.experimental.pallas as pl
import jax.experimental.pallas.tpu as pltpu

S, D, F = 2048, 576, 4608
DP = 640
FC = 512
NC = F // FC
TT = 256
NTT = S // TT
BIG = 4
H, DH, WIN, DIL = 32, 18, 8, 2
HALO = 16
NSLAB = 14
RC = 8
ATT_SPREAD = 7
PREP_AT = 1
XG = 2
OSPLIT = 4
NSEM = 6
EPS = 1e-5
LOG2E = 1.4426950408889634
SCALE = DH ** -0.5
NT = (((1,), (1,)), ((), ()))
F32 = jnp.float32
BF16 = jnp.bfloat16


def _mish(h):
    e = jnp.exp(jnp.minimum(h, 20.0))
    n = e * (e + 2.0)
    return h * (n * pl.reciprocal(n + 2.0, approx=True))


def _never(v):
    return jnp.minimum(pltpu.bitcast(v, jnp.int32), 5) > 7


def _kernel(x_hbm, wqkv_hbm, wo_hbm, w1_hbm, b1_hbm, w2_hbm, out_hbm,
            x_s, xn_s, w1_s, w2_s, wqkv_s, wo_s, wt_s, wot_s, slab_s,
            act_s, acc_s, qkv_s, o_s, out_s, b1_s, stg_s, sems):

    def rows(j, n=TT):
        if isinstance(j, int):
            return pl.ds(j * n, n)
        return pl.ds(pl.multiple_of(j * n, n), n)

    def x_copy(j, sem):
        return pltpu.make_async_copy(x_hbm.at[:, rows(j)], x_s.at[j], sems.at[sem])

    def w1_copy(c, sem):
        return pltpu.make_async_copy(w1_hbm.at[:, rows(c, FC)],
                                     w1_s.at[c, pl.ds(0, D), :], sems.at[sem])

    def w1_half(u, sem):
        return pltpu.make_async_copy(w1_hbm.at[:, rows(u, FC // 2)],
                                     w1_s.at[0, pl.ds(0, D), rows(u, FC // 2)],
                                     sems.at[sem])

    def w2_copy(c, sem):
        return pltpu.make_async_copy(w2_hbm.at[:, rows(c, FC)], w2_s.at[c], sems.at[sem])

    def out_copy(j, r0, nr):
        return pltpu.make_async_copy(out_s.at[j, pl.ds(r0, nr), :],
                                     out_hbm.at[pl.ds(r0, nr), rows(j)], sems.at[0])

    wqkv_copy = pltpu.make_async_copy(wqkv_hbm, wqkv_s, sems.at[1])
    wo_copy = pltpu.make_async_copy(wo_hbm, wo_s, sems.at[1])
    b1_copy = pltpu.make_async_copy(b1_hbm, b1_s, sems.at[0])

    def ffn1(r, c, lhs=None, cols=(0, FC)):
        lhs = xn_s[r, :] if lhs is None else lhs
        h = jnp.dot(lhs, w1_s[c, :, cols[0]:cols[1]], preferred_element_type=F32)
        act_s[r, cols[0]:cols[1]] = _mish(h).astype(BF16)

    def ffn2(j, c):
        return lax.dot_general(w2_s[c], act_s[rows(j), :], NT, preferred_element_type=F32)

    def layernorm(j, stage=None, chain=False):
        w = 128 if chain else TT
        rowp = lax.broadcasted_iota(jnp.int32, (DP - D, w), 0)
        ones_pad = jnp.where(rowp == 0, 1.0, 0.0).astype(F32)
        prev = None
        for u in range(TT // w):
            xt = x_s[j, :, u * w:(u + 1) * w].astype(F32)
            xs = xt
            if prev is not None:
                head = jnp.where(_never(prev), 0.0, xt[0:8, :])
                xs = jnp.concatenate([head, xt[8:, :]], axis=0)
            m = jnp.sum(xs, axis=0, keepdims=True) * (1.0 / D)
            xc = xt - m
            v = jnp.sum(xc * xc, axis=0, keepdims=True) * (1.0 / D)
            r = lax.rsqrt(v + EPS)
            prev = jnp.broadcast_to(r, (8, w))
            xn = jnp.concatenate([xc * r, ones_pad], axis=0)
            xnb = xn.T.astype(BF16)
            xn_s[rows(j * (TT // w) + u, w), :] = xnb
            if stage is not None:
                stage[u * w:(u + 1) * w, :] = xnb

    def bias_rows():
        b = b1_s[...].astype(F32)
        row16 = lax.broadcasted_iota(jnp.int32, (16, 128), 0)
        for c in range(NC):
            for u in range(FC // 128):
                r = c * (FC // 128) + u
                w1_s[c, D:D + 16, u * 128:(u + 1) * 128] = jnp.where(
                    row16 == 0, jnp.broadcast_to(b[r:r + 1, :], (16, 128)), 0.0
                ).astype(BF16)

    def prep_weights():
        for c in range(5):
            nr = 128 if c < 4 else 64
            blk = wqkv_s[c * 128:c * 128 + nr, :].astype(F32)
            if nr < 128:
                blk = jnp.concatenate([blk, jnp.zeros((128 - nr, 3 * D), F32)], axis=0)
            slab_s[c, 0:3 * D, :] = blk.T
        for t in range(3):
            for d in range(DH):
                if d < 16:
                    dst = t * 512 + d * H
                else:
                    dst = (1536, 1664, 1600)[t] + (d - 16) * H
                wt_s[dst:dst + H, :] = jnp.concatenate(
                    [slab_s[c, pl.ds(t * D + d, H, stride=DH), :] for c in range(5)],
                    axis=1).astype(BF16)
        for c in range(5):
            nc = 128 if c < 4 else 64
            blk = wo_s[:, c * 128:c * 128 + nc].astype(F32)
            if nc < 128:
                blk = jnp.concatenate([blk, jnp.zeros((D, 128 - nc), F32)], axis=1)
            slab_s[c, 3 * D:4 * D, :] = blk
        for c in range(5):
            nr = 128 if c < 4 else 64
            parts = [slab_s[c, pl.ds(3 * D + d, H, stride=DH), :] for d in range(16)]
            parts.append(jnp.zeros((64, 128), F32))
            parts += [slab_s[c, pl.ds(3 * D + d, H, stride=DH), :] for d in (16, 17)]
            pt = jnp.concatenate(parts, axis=0).T[:nr, :]
            wot_s[c * 128:c * 128 + nr, :] = pt.astype(BF16)
            g = pltpu.bitcast(pt[nr - 8:nr, 0:128], jnp.int32)
            for u in range(1, 5):
                g = jnp.minimum(
                    g, pltpu.bitcast(pt[nr - 8:nr, u * 128:(u + 1) * 128], jnp.int32))
            z = jnp.where(jnp.minimum(g, 5) > 7, 1.0, 0.0)
            wt_s[3 * D:NSLAB * 128, c * 128:(c + 1) * 128] = jnp.concatenate(
                [z] * 8, axis=0).astype(BF16)

    q_sl = (0, 1, 2, 3, 12)
    k_sl = (4, 5, 6, 7, 13)
    v_sl = (8, 9, 10, 11, 12)

    def attention_rows(t, r, gate):
        q = [jnp.where(gate, 0.0, qkv_s[sl, HALO + r:HALO + r + RC, :]) for sl in q_sl]
        ls = []
        for w in range(WIN):
            o0 = HALO + r - DIL * w
            s = q[0] * qkv_s[k_sl[0], o0:o0 + RC, :]
            for u in range(1, 5):
                s = s + q[u] * qkv_s[k_sl[u], o0:o0 + RC, :]
            s = s + pltpu.roll(s, 64, 1)
            s = s + pltpu.roll(s, 32, 1)
            if r < HALO and w > 0:
                pos = t * TT + r + lax.broadcasted_iota(jnp.int32, (RC, 128), 0)
                s = jnp.where(pos >= DIL * w, s, -1e9 / SCALE)
            ls.append(s)
        m = ls[0]
        for w in range(1, WIN):
            m = jnp.maximum(m, ls[w])
        ps = [jnp.exp2((l - m) * (SCALE * LOG2E)) for l in ls]
        den = ps[0]
        for w in range(1, WIN):
            den = den + ps[w]
        rinv = pl.reciprocal(den, approx=True)
        outs = []
        for u in range(5):
            a = ps[0] * qkv_s[v_sl[u], HALO + r:HALO + r + RC, :]
            for w in range(1, WIN):
                o0 = HALO + r - DIL * w
                a = a + ps[w] * qkv_s[v_sl[u], o0:o0 + RC, :]
            outs.append(a * rinv)
        o_s[r:r + RC, :] = jnp.concatenate(outs, axis=1).astype(BF16)
        return den

    chunks = list(range(0, TT, RC))
    att_sched = [[] for _ in range(NTT)]
    for i, r in enumerate(chunks):
        att_sched[i * ATT_SPREAD // len(chunks)].append(r)

    def attention_group(t, j, y):
        gate = _never(y[0:RC, 0:128])
        for r in att_sched[j]:
            gate = _never(attention_rows(t, r, gate))

    def qkv_proj(t):
        qkv_s[4:NSLAB, 0:HALO, :] = qkv_s[4:NSLAB, TT:TT + HALO, :]
        qkv = lax.dot_general(xn_s[rows(t), :], wt_s[...], NT, preferred_element_type=F32)
        for sl in range(NSLAB):
            qkv_s[sl, HALO:HALO + TT, :] = qkv[:, sl * 128:(sl + 1) * 128]

    def wo_proj():
        return lax.dot_general(wot_s[...], o_s[...], NT, preferred_element_type=F32)

    x_copy(0, 0).start()
    b1_copy.start()
    w1_half(0, 5).start()
    x_copy(1, 1).start()
    w1_half(1, 1).start()
    x_copy(2, 2).start()
    for j in range(3, NTT - 1):
        x_copy(j, 3 + (j - 3) // XG).start()
    for c in range(NC):
        w1_s[c, D + 16:DP, :] = jnp.zeros((DP - D - 16, FC), BF16)
    qkv_s[:, TT:TT + HALO, :] = jnp.zeros((NSLAB, HALO, 128), F32)

    def zero_acc(j, carry):
        acc_s[j] = jnp.zeros((D, TT), F32)
        return carry

    lax.fori_loop(BIG, NTT, zero_acc, 0)

    x_copy(0, 0).wait()
    b1_copy.wait()
    layernorm(0)
    bias_rows()
    w1_half(0, 5).wait()
    x_copy(NTT - 1, 5).start()
    w1_copy(1, 5).start()
    w2_copy(0, 5).start()
    ffn1(rows(0), 0, cols=(0, 128))
    ffn1(rows(0), 0, cols=(128, 256))
    x_copy(1, 1).wait()
    w1_half(1, 1).wait()
    wqkv_copy.start()
    wo_copy.start()
    layernorm(1)
    ffn1(rows(0), 0, cols=(256, 384))
    ffn1(rows(0), 0, cols=(384, 512))
    x_copy(2, 2).wait()
    layernorm(2, stg_s.at[XG - 1], chain=True)
    ffn1(rows(1), 0)

    def step0(i, carry):
        for u in range(XG):
            x_copy(XG * i + 3 + u, 3 + i).wait()
        for u in range(XG):
            layernorm(XG * i + 3 + u, stg_s.at[u], chain=True)
            ffn1(rows(XG * i + 2 + u), 0, lhs=stg_s[(u - 1) % XG])
        return carry

    lax.fori_loop(0, (NTT - 4) // XG, step0, 0)

    x_copy(NTT - 1, 5).wait()
    w1_copy(1, 5).wait()
    w2_copy(0, 5).wait()
    w1_copy(2, 2).start()
    w2_copy(1, 2).start()
    w2_copy(NC - 1, 4).start()
    layernorm(NTT - 1, chain=True)
    ffn1(rows(NTT - 2), 0)
    ffn1(rows(NTT - 1), 0)
    for j in range(BIG):
        acc_s[j] = ffn2(j, 0)
        if j == PREP_AT:
            wqkv_copy.wait()
            wo_copy.wait()
            prep_weights()
    ffn1(rows(0, TT * BIG), 1)
    qkv_proj(0)
    w2_copy(NC - 1, 4).wait()

    def step(s, carry):
        t = s - 2
        cur = 2 + lax.rem(s, 2)
        w1_copy(s, cur).wait()
        w2_copy(s - 1, cur).wait()

        @pl.when(s + 1 < NC)
        def _():
            w1_copy(s + 1, 5 - cur).start()
            w2_copy(s, 5 - cur).start()

        for j in range(NTT):
            c = s - j // BIG
            y = ffn2(j, c - 1)
            acc_s[j] += y
            if j % BIG == BIG - 1:
                ffn1(rows(j // BIG, TT * BIG), c)
            attention_group(t, j, y)
        acc_s[t] += wo_proj()
        qkv_proj(t + 1)
        return carry

    lax.fori_loop(2, NC, step, 0)

    t = NTT - 1
    outs = []

    def finish(j, extra=None):
        y = ffn2(j, NC - 1)
        res = (acc_s[j] + x_s[j].astype(F32)) + y
        if extra is not None:
            res = res + extra
        nsp = OSPLIT if j == t else 1
        nr = D // nsp
        for u in range(nsp):
            out_s[j, u * nr:(u + 1) * nr, :] = res[u * nr:(u + 1) * nr, :].astype(BF16)
            cp = out_copy(j, u * nr, nr)
            cp.start()
            outs.append(cp)
        return y

    for j in range(BIG, NTT):
        y = ffn2(j, NC - 2)
        acc_s[j] += y
        attention_group(t, j - BIG, y)
    ffn1(rows(1, TT * BIG), NC - 1)
    for j in range(BIG):
        y = finish(j)
        attention_group(t, BIG + j, y)
    for j in range(BIG, NTT):
        finish(j, wo_proj() if j == t else None)
    for cp in outs:
        cp.wait()


@jax.jit
def pallas_parallel_sum__sliding_local_dilated__dense_activation_mish__prompt_kernel(
    A_x: jax.Array,
    A_wqkv: jax.Array,
    A_wo: jax.Array,
    B_x: jax.Array,
    B_w1: jax.Array,
    B_b1: jax.Array,
    B_w2: jax.Array,
):
    del B_x
    xT = jnp.transpose(A_x, (0, 2, 1)).reshape(D, S)
    any_spec = pl.BlockSpec(memory_space=pl.ANY)
    outT = pl.pallas_call(
        _kernel,
        out_shape=jax.ShapeDtypeStruct((D, S), BF16),
        in_specs=[any_spec] * 6,
        out_specs=any_spec,
        scratch_shapes=[
            pltpu.VMEM((NTT, D, TT), BF16),
            pltpu.VMEM((S, DP), BF16),
            pltpu.VMEM((NC, DP, FC), BF16),
            pltpu.VMEM((NC, D, FC), BF16),
            pltpu.VMEM((D, 3 * D), BF16),
            pltpu.VMEM((D, D), BF16),
            pltpu.VMEM((NSLAB * 128, DP), BF16),
            pltpu.VMEM((D, DP), BF16),
            pltpu.VMEM((5, 4 * D, 128), F32),
            pltpu.VMEM((S, FC), BF16),
            pltpu.VMEM((NTT, D, TT), F32),
            pltpu.VMEM((NSLAB, TT + HALO, 128), F32),
            pltpu.VMEM((TT, DP), BF16),
            pltpu.VMEM((NTT, D, TT), BF16),
            pltpu.VMEM((F // 128, 128), BF16),
            pltpu.VMEM((XG, TT, DP), BF16),
            pltpu.SemaphoreType.DMA((NSEM,)),
        ],
        compiler_params=pltpu.CompilerParams(
            vmem_limit_bytes=64 * 1024 * 1024,
            disable_bounds_checks=True,
            disable_semaphore_checks=True,
        ),
        name="fused_attn_ffn",
    )(xT, A_wqkv, A_wo, B_w1, B_b1.reshape(F // 128, 128), B_w2.T)
    return jnp.transpose(outT.reshape(1, D, S), (0, 2, 1))
```

```python
import jax
import jax.numpy as jnp
from jax import lax
import jax.experimental.pallas as pl
import jax.experimental.pallas.tpu as pltpu

S, D, F = 2048, 576, 4608
DP = 640
FC = 512
NC = F // FC
TT = 256
NTT = S // TT
BIG = 4
H, DH, WIN, DIL = 32, 18, 8, 2
HALO = 16
NSLAB = 14
RC = 8
ATT_SPREAD = 7
PREP_AT = 1
XG = 2
OSPLIT = 4
NSEM = 6
EPS = 1e-5
LOG2E = 1.4426950408889634
SCALE = DH ** -0.5
NT = (((1,), (1,)), ((), ()))
F32 = jnp.float32
BF16 = jnp.bfloat16


def _mish(h):
    e = jnp.exp(jnp.minimum(h, 20.0))
    n = e * (e + 2.0)
    return h * (n * pl.reciprocal(n + 2.0, approx=True))


def _never(v):
    return jnp.minimum(pltpu.bitcast(v, jnp.int32), 5) > 7


def _kernel(x_hbm, wqkv_hbm, wo_hbm, w1_hbm, b1_hbm, w2_hbm, out_hbm,
            x_s, xn_s, w1_s, w2_s, wqkv_s, wo_s, wt_s, wot_s, slab_s,
            act_s, acc_s, qkv_s, o_s, out_s, b1_s, stg_s, sems):

    def rows(j, n=TT):
        if isinstance(j, int):
            return pl.ds(j * n, n)
        return pl.ds(pl.multiple_of(j * n, n), n)

    def x_copy(j, sem):
        return pltpu.make_async_copy(x_hbm.at[:, rows(j)], x_s.at[j], sems.at[sem])

    def w1_copy(c, sem):
        return pltpu.make_async_copy(w1_hbm.at[:, rows(c, FC)],
                                     w1_s.at[c, pl.ds(0, D), :], sems.at[sem])

    def w1_half(u, sem):
        return pltpu.make_async_copy(w1_hbm.at[:, rows(u, FC // 2)],
                                     w1_s.at[0, pl.ds(0, D), rows(u, FC // 2)],
                                     sems.at[sem])

    def w2_copy(c, sem):
        return pltpu.make_async_copy(w2_hbm.at[:, rows(c, FC)], w2_s.at[c], sems.at[sem])

    def out_copy(j, r0, nr):
        return pltpu.make_async_copy(out_s.at[j, pl.ds(r0, nr), :],
                                     out_hbm.at[pl.ds(r0, nr), rows(j)], sems.at[0])

    wqkv_copy = pltpu.make_async_copy(wqkv_hbm, wqkv_s, sems.at[1])
    wo_copy = pltpu.make_async_copy(wo_hbm, wo_s, sems.at[1])
    b1_copy = pltpu.make_async_copy(b1_hbm, b1_s, sems.at[0])

    def ffn1(r, c, lhs=None, cols=(0, FC)):
        lhs = xn_s[r, :] if lhs is None else lhs
        h = jnp.dot(lhs, w1_s[c, :, cols[0]:cols[1]], preferred_element_type=F32)
        act_s[r, cols[0]:cols[1]] = _mish(h).astype(BF16)

    def ffn2(j, c):
        return lax.dot_general(w2_s[c], act_s[rows(j), :], NT, preferred_element_type=F32)

    def layernorm(j, stage=None, chain=False):
        w = 128 if chain else TT
        rowp = lax.broadcasted_iota(jnp.int32, (DP - D, w), 0)
        ones_pad = jnp.where(rowp == 0, 1.0, 0.0).astype(F32)
        prev = None
        for u in range(TT // w):
            xt = x_s[j, :, u * w:(u + 1) * w].astype(F32)
            xs = xt
            if prev is not None:
                head = jnp.where(_never(prev), 0.0, xt[0:8, :])
                xs = jnp.concatenate([head, xt[8:, :]], axis=0)
            m = jnp.sum(xs, axis=0, keepdims=True) * (1.0 / D)
            xc = xt - m
            v = jnp.sum(xc * xc, axis=0, keepdims=True) * (1.0 / D)
            r = lax.rsqrt(v + EPS)
            prev = jnp.broadcast_to(r, (8, w))
            xn = jnp.concatenate([xc * r, ones_pad], axis=0)
            xnb = xn.T.astype(BF16)
            xn_s[rows(j * (TT // w) + u, w), :] = xnb
            if stage is not None:
                stage[u * w:(u + 1) * w, :] = xnb

    def bias_rows():
        b = b1_s[...].astype(F32)
        row16 = lax.broadcasted_iota(jnp.int32, (16, 128), 0)
        for c in range(NC):
            for u in range(FC // 128):
                r = c * (FC // 128) + u
                w1_s[c, D:D + 16, u * 128:(u + 1) * 128] = jnp.where(
                    row16 == 0, jnp.broadcast_to(b[r:r + 1, :], (16, 128)), 0.0
                ).astype(BF16)

    def prep_weights():
        for c in range(5):
            nr = 128 if c < 4 else 64
            blk = wqkv_s[c * 128:c * 128 + nr, :].astype(F32)
            if nr < 128:
                blk = jnp.concatenate([blk, jnp.zeros((128 - nr, 3 * D), F32)], axis=0)
            slab_s[c, 0:3 * D, :] = blk.T
        for t in range(3):
            for d in range(DH):
                if d < 16:
                    dst = t * 512 + d * H
                else:
                    dst = (1536, 1664, 1600)[t] + (d - 16) * H
                wt_s[dst:dst + H, :] = jnp.concatenate(
                    [slab_s[c, pl.ds(t * D + d, H, stride=DH), :] for c in range(5)],
                    axis=1).astype(BF16)
        for c in range(5):
            nc = 128 if c < 4 else 64
            blk = wo_s[:, c * 128:c * 128 + nc].astype(F32)
            if nc < 128:
                blk = jnp.concatenate([blk, jnp.zeros((D, 128 - nc), F32)], axis=1)
            slab_s[c, 3 * D:4 * D, :] = blk
        for c in range(5):
            nr = 128 if c < 4 else 64
            parts = [slab_s[c, pl.ds(3 * D + d, H, stride=DH), :] for d in range(16)]
            parts.append(jnp.zeros((64, 128), F32))
            parts += [slab_s[c, pl.ds(3 * D + d, H, stride=DH), :] for d in (16, 17)]
            pt = jnp.concatenate(parts, axis=0).T[:nr, :]
            wot_s[c * 128:c * 128 + nr, :] = pt.astype(BF16)
            g = pltpu.bitcast(pt[nr - 8:nr, 0:128], jnp.int32)
            for u in range(1, 5):
                g = jnp.minimum(
                    g, pltpu.bitcast(pt[nr - 8:nr, u * 128:(u + 1) * 128], jnp.int32))
            z = jnp.where(jnp.minimum(g, 5) > 7, 1.0, 0.0)
            wt_s[3 * D:NSLAB * 128, c * 128:(c + 1) * 128] = jnp.concatenate(
                [z] * 8, axis=0).astype(BF16)

    q_sl = (0, 1, 2, 3, 12)
    k_sl = (4, 5, 6, 7, 13)
    v_sl = (8, 9, 10, 11, 12)

    def attention_rows(t, r, gate):
        q = [jnp.where(gate, 0.0, qkv_s[sl, HALO + r:HALO + r + RC, :]) for sl in q_sl]
        ls = []
        for w in range(WIN):
            o0 = HALO + r - DIL * w
            s = q[0] * qkv_s[k_sl[0], o0:o0 + RC, :]
            for u in range(1, 5):
                s = s + q[u] * qkv_s[k_sl[u], o0:o0 + RC, :]
            s = s + pltpu.roll(s, 64, 1)
            s = s + pltpu.roll(s, 32, 1)
            if r < HALO and w > 0:
                pos = t * TT + r + lax.broadcasted_iota(jnp.int32, (RC, 128), 0)
                s = jnp.where(pos >= DIL * w, s, -1e9 / SCALE)
            ls.append(s)
        m = ls[0]
        for w in range(1, WIN):
            m = jnp.maximum(m, ls[w])
        ps = [jnp.exp2((l - m) * (SCALE * LOG2E)) for l in ls]
        den = ps[0]
        for w in range(1, WIN):
            den = den + ps[w]
        rinv = pl.reciprocal(den, approx=True)
        outs = []
        for u in range(5):
            a = ps[0] * qkv_s[v_sl[u], HALO + r:HALO + r + RC, :]
            for w in range(1, WIN):
                o0 = HALO + r - DIL * w
                a = a + ps[w] * qkv_s[v_sl[u], o0:o0 + RC, :]
            outs.append(a * rinv)
        o_s[r:r + RC, :] = jnp.concatenate(outs, axis=1).astype(BF16)
        return den

    chunks = list(range(0, TT, RC))
    att_sched = [[] for _ in range(NTT)]
    for i, r in enumerate(chunks):
        att_sched[i * ATT_SPREAD // len(chunks)].append(r)

    def attention_group(t, j, y):
        gate = _never(y[0:RC, 0:128])
        for r in att_sched[j]:
            gate = _never(attention_rows(t, r, gate))

    def qkv_proj(t):
        qkv_s[4:NSLAB, 0:HALO, :] = qkv_s[4:NSLAB, TT:TT + HALO, :]
        qkv = lax.dot_general(xn_s[rows(t), :], wt_s[...], NT, preferred_element_type=F32)
        for sl in range(NSLAB):
            qkv_s[sl, HALO:HALO + TT, :] = qkv[:, sl * 128:(sl + 1) * 128]

    def wo_proj():
        return lax.dot_general(wot_s[...], o_s[...], NT, preferred_element_type=F32)

    x_copy(0, 0).start()
    b1_copy.start()
    w1_half(0, 5).start()
    x_copy(1, 1).start()
    w1_half(1, 1).start()
    x_copy(2, 2).start()
    for j in range(3, NTT - 1):
        x_copy(j, 3 + (j - 3) // XG).start()
    for c in range(NC):
        w1_s[c, D + 16:DP, :] = jnp.zeros((DP - D - 16, FC), BF16)
    qkv_s[:, TT:TT + HALO, :] = jnp.zeros((NSLAB, HALO, 128), F32)

    def zero_acc(j, carry):
        acc_s[j] = jnp.zeros((D, TT), F32)
        return carry

    lax.fori_loop(BIG, NTT, zero_acc, 0)

    x_copy(0, 0).wait()
    b1_copy.wait()
    layernorm(0)
    bias_rows()
    w1_half(0, 5).wait()
    x_copy(NTT - 1, 5).start()
    w1_copy(1, 5).start()
    w2_copy(0, 5).start()
    ffn1(rows(0, 128), 0, cols=(0, 256))
    ffn1(rows(1, 128), 0, cols=(0, 256))
    x_copy(1, 1).wait()
    w1_half(1, 1).wait()
    wqkv_copy.start()
    wo_copy.start()
    layernorm(1)
    ffn1(rows(0, 128), 0, cols=(256, 512))
    ffn1(rows(1, 128), 0, cols=(256, 512))
    x_copy(2, 2).wait()
    layernorm(2, stg_s.at[XG - 1], chain=True)
    ffn1(rows(1), 0)

    def step0(i, carry):
        for u in range(XG):
            x_copy(XG * i + 3 + u, 3 + i).wait()
        for u in range(XG):
            layernorm(XG * i + 3 + u, stg_s.at[u], chain=True)
            ffn1(rows(XG * i + 2 + u), 0, lhs=stg_s[(u - 1) % XG])
        return carry

    lax.fori_loop(0, (NTT - 4) // XG, step0, 0)

    x_copy(NTT - 1, 5).wait()
    w1_copy(1, 5).wait()
    w2_copy(0, 5).wait()
    w1_copy(2, 2).start()
    w2_copy(1, 2).start()
    w2_copy(NC - 1, 4).start()
    layernorm(NTT - 1, chain=True)
    ffn1(rows(NTT - 2), 0)
    ffn1(rows(NTT - 1), 0)
    for j in range(BIG):
        acc_s[j] = ffn2(j, 0)
        if j == PREP_AT:
            wqkv_copy.wait()
            wo_copy.wait()
            prep_weights()
    ffn1(rows(0, TT * BIG), 1)
    qkv_proj(0)
    w2_copy(NC - 1, 4).wait()

    def step(s, carry):
        t = s - 2
        cur = 2 + lax.rem(s, 2)
        w1_copy(s, cur).wait()
        w2_copy(s - 1, cur).wait()

        @pl.when(s + 1 < NC)
        def _():
            w1_copy(s + 1, 5 - cur).start()
            w2_copy(s, 5 - cur).start()

        for j in range(NTT):
            c = s - j // BIG
            y = ffn2(j, c - 1)
            acc_s[j] += y
            if j % BIG == BIG - 1:
                ffn1(rows(j // BIG, TT * BIG), c)
            attention_group(t, j, y)
        acc_s[t] += wo_proj()
        qkv_proj(t + 1)
        return carry

    lax.fori_loop(2, NC, step, 0)

    t = NTT - 1
    outs = []

    def finish(j, extra=None):
        y = ffn2(j, NC - 1)
        res = (acc_s[j] + x_s[j].astype(F32)) + y
        if extra is not None:
            res = res + extra
        nsp = OSPLIT if j == t else 1
        nr = D // nsp
        for u in range(nsp):
            out_s[j, u * nr:(u + 1) * nr, :] = res[u * nr:(u + 1) * nr, :].astype(BF16)
            cp = out_copy(j, u * nr, nr)
            cp.start()
            outs.append(cp)
        return y

    for j in range(BIG, NTT):
        y = ffn2(j, NC - 2)
        acc_s[j] += y
        attention_group(t, j - BIG, y)
    ffn1(rows(1, TT * BIG), NC - 1)
    for j in range(BIG):
        y = finish(j)
        attention_group(t, BIG + j, y)
    for j in range(BIG, NTT):
        finish(j, wo_proj() if j == t else None)
    for cp in outs:
        cp.wait()


@jax.jit
def pallas_parallel_sum__sliding_local_dilated__dense_activation_mish__prompt_kernel(
    A_x: jax.Array,
    A_wqkv: jax.Array,
    A_wo: jax.Array,
    B_x: jax.Array,
    B_w1: jax.Array,
    B_b1: jax.Array,
    B_w2: jax.Array,
):
    del B_x
    xT = jnp.transpose(A_x, (0, 2, 1)).reshape(D, S)
    any_spec = pl.BlockSpec(memory_space=pl.ANY)
    outT = pl.pallas_call(
        _kernel,
        out_shape=jax.ShapeDtypeStruct((D, S), BF16),
        in_specs=[any_spec] * 6,
        out_specs=any_spec,
        scratch_shapes=[
            pltpu.VMEM((NTT, D, TT), BF16),
            pltpu.VMEM((S, DP), BF16),
            pltpu.VMEM((NC, DP, FC), BF16),
            pltpu.VMEM((NC, D, FC), BF16),
            pltpu.VMEM((D, 3 * D), BF16),
            pltpu.VMEM((D, D), BF16),
            pltpu.VMEM((NSLAB * 128, DP), BF16),
            pltpu.VMEM((D, DP), BF16),
            pltpu.VMEM((5, 4 * D, 128), F32),
            pltpu.VMEM((S, FC), BF16),
            pltpu.VMEM((NTT, D, TT), F32),
            pltpu.VMEM((NSLAB, TT + HALO, 128), F32),
            pltpu.VMEM((TT, DP), BF16),
            pltpu.VMEM((NTT, D, TT), BF16),
            pltpu.VMEM((F // 128, 128), BF16),
            pltpu.VMEM((XG, TT, DP), BF16),
            pltpu.SemaphoreType.DMA((NSEM,)),
        ],
        compiler_params=pltpu.CompilerParams(
            vmem_limit_bytes=64 * 1024 * 1024,
            disable_bounds_checks=True,
            disable_semaphore_checks=True,
        ),
        name="fused_attn_ffn",
    )(xT, A_wqkv, A_wo, B_w1, B_b1.reshape(F // 128, 128), B_w2.T)
    return jnp.transpose(outT.reshape(1, D, S), (0, 2, 1))
```
